```python
import os as _os
_os.environ.setdefault("JAX_PLATFORMS", "cpu")
import jax
import jax.numpy as jnp

def _softmax(x, axis=-1):
    return jax.nn.softmax(x, axis=axis)
def _gelu(x):
    return jax.nn.gelu(x, approximate=True)
def _silu(x):
    return jax.nn.silu(x)
def _sigmoid(x):
    return jax.nn.sigmoid(x)
def _layernorm(x, axis=-1, eps=1e-5):
    m = jnp.mean(x, axis=axis, keepdims=True)
    v = jnp.var(x, axis=axis, keepdims=True)
    return (x - m) / jnp.sqrt(v + eps)
def _scatter_add(tgt, idx, src, axis=0):
    return tgt.at[idx].add(src)
def _segment_sum(src, seg, n):
    return jax.ops.segment_sum(src, seg, n)
class _Rng:
    def __init__(self, key):
        self._k = key
    def _next(self):
        self._k, sub = jax.random.split(self._k)
        return sub
    def normal(self, shape):
        return jax.random.normal(self._next(), shape, dtype=jnp.bfloat16)
    def randint(self, lo, hi, shape):
        return jax.random.randint(self._next(), shape, lo, hi, dtype=jnp.int32)
    def uniform(self, shape, lo=0.0, hi=1.0):
        return jax.random.uniform(self._next(), shape, jnp.bfloat16, lo, hi)
    def permutation(self, n):
        return jax.random.permutation(self._next(), n)


kernel_name = 'sequential_preLN__ssm_conv_h3__mixer_channel_mlp__prompt'

def setup_inputs():
    _rng = _Rng(jax.random.key(int.from_bytes(__import__("os").urandom(4), "little")))
    _w = (lambda a: (lambda t: t.astype(jnp.bfloat16) if jnp.issubdtype(t.dtype, jnp.floating) else t)(jnp.asarray(a)))
    def _A_setup():
        B, S, D = 1, 2048, 448
        ks = 4
        return {
            "q": _w((lambda *s: _rng.normal(s) * 0.05)(B, S, D)),
            "k": _w((lambda *s: _rng.normal(s) * 0.05)(B, S, D)),
            "v": _w((lambda *s: _rng.normal(s) * 0.05)(B, S, D)),
            "shift_k": _w((lambda *s: _rng.normal(s) * 0.05)(D, ks) * 0.5),
            "ssm_k": _w((lambda *s: _rng.normal(s) * 0.05)(D, S) * (1.0 / S ** 0.5)),
            "ssm_D": _w((lambda *s: _rng.normal(s) * 0.05)(D)),
        }
    _A_in = _A_setup()

    def _B_setup():
        B, S, D, F = 1, 2048, 448, 1792
        return {
            "x": _w((lambda *s: _rng.normal(s) * 0.05)(B, S, D)),
            "w1": _w((lambda *s: _rng.normal(s) * 0.2)(D, F) * (D ** -0.5)),
            "b1": _w((lambda *s: _rng.normal(s) * 0.2)(F)),
            "w2": _w((lambda *s: _rng.normal(s) * 0.2)(F, D) * (F ** -0.5)),
            "b2": _w((lambda *s: _rng.normal(s) * 0.05)(D)),
        }
    _B_in = _B_setup()

    return {
        "A_q": _A_in["q"],
        "A_k": _A_in["k"],
        "A_v": _A_in["v"],
        "A_shift_k": _A_in["shift_k"],
        "A_ssm_k": _A_in["ssm_k"],
        "A_ssm_D": _A_in["ssm_D"],
        "B_x": _B_in["x"],
        "B_w1": _B_in["w1"],
        "B_b1": _B_in["b1"],
        "B_w2": _B_in["w2"],
        "B_b2": _B_in["b2"],
    }

def reference(A_q, A_k, A_v, A_shift_k, A_ssm_k, A_ssm_D, B_x, B_w1, B_b1, B_w2, B_b2):
    def _A_ref(q, k, v, shift_k, ssm_k, ssm_D):
        B, S, D = q.shape
        ks = shift_k.shape[-1]
        k_pad = jnp.pad(k, ((0, 0), (ks - 1, 0), (0, 0)))
        k_shift = jnp.zeros_like(k)
        for t in range(ks):
            k_shift = k_shift + k_pad[:, t:t + S, :] * shift_k[:, ks - 1 - t][None, None, :]
        kv = k_shift * v
        L = 2 * S
        kv_pad = jnp.pad(kv, ((0, 0), (0, S), (0, 0)))
        kf_pad = jnp.pad(ssm_k, ((0, 0), (0, S)))
        kv_f = (lambda x, axes=(-2,-1): jnp.fft.rfft2(x.astype(jnp.float32), axes=axes))(kv_pad[:, None, :, :], axes=(1, 2))
        kf_f = (lambda x, axes=(-2,-1): jnp.fft.rfft2(x.astype(jnp.float32), axes=axes))(kf_pad[:, None, :], axes=(1, 2))
        kf_f = (lambda x, *d: x.transpose(*d))(kf_f, 1, 2, 0)
        y_f = kv_f * kf_f[None, :, :, :]
        y = (lambda x, s, axes=(-2,-1): jnp.fft.irfft2(x, s=s, axes=axes).astype(jnp.bfloat16))(y_f, (1, L), axes=(1, 2))[:, 0, :S, :]
        y = y + kv * ssm_D[None, None, :]
        return q * y

    def _B_ref(x, w1, b1, w2, b2):
        y = _layernorm(x, axis=-1)
        h = _gelu(jnp.einsum("bsd,df->bsf", y, w1) + b1)
        return jnp.einsum("bsf,fd->bsd", h, w2) + b2

    x = A_q
    h = x + _A_ref(_layernorm(x, axis=-1), A_k, A_v, A_shift_k, A_ssm_k, A_ssm_D)
    h2 = h + _B_ref(_layernorm(h, axis=-1), B_w1, B_b1, B_w2, B_b2)
    return h2
```

```python
import numpy as np
import jax
import jax.numpy as jnp
import jax.experimental.pallas as pl
import jax.experimental.pallas.tpu as pltpu

S, D, F = 2048, 448, 1792
B = 512
R = 4
NC = S // B
KP = 512
FC = 128
NF = F // FC
RT = 16
NT = D // RT
H = RT // 2
GB = [112] * 4
GD = [112] * 4
G0 = [64, 64, 48, 48, 64, 64, 48, 48]
ORDER0 = 'a0 a1 c0 a2 c1 a3 | c2 a4 c3 a5 c4 a6 c5 a7 c6 c7'
EPS = 1e-5
f32 = jnp.float32
bf16 = jnp.bfloat16
u32 = jnp.uint32
C1 = 0.7978845608028654
C2 = C1 * 0.044715
SK, SU, SR = 0, 8, 16
HL = 25 * 128
POS_C1 = 7
POS_AB = [9, 3, 3]
POS_FAB = [9, 3, 3]
POS_D = [18, 21, 21]
POS_FD = 19
WP = [((0, 4), (0, 3)), ((4, 7), (3, 6)), ((7, 11), (6, 10)), ((11, 14), (10, 14))]


def _cos2048(x):
    n = x - 2048.0 * jnp.floor(x * (1.0 / 2048.0))
    u = jnp.abs(n - 1024.0) * (1.0 / 512.0) - 1.0
    u2 = u * u
    pl_ = 1.6044118478735982e-04
    for cf in (-4.681754135318688e-03, 7.969262624616703e-02, -6.459640975062462e-01, 1.5707963267948966):
        pl_ = pl_ * u2 + cf
    return pl_ * u


def _sample_index(b, p):
    r = (b - p) & 3
    return 128 * r + ((b - r) & 127)


def _bfly(e, sign):
    ar, ai = e[0][0] + e[2][0], e[0][1] + e[2][1]
    br, bi = e[0][0] - e[2][0], e[0][1] - e[2][1]
    cr, ci = e[1][0] + e[3][0], e[1][1] + e[3][1]
    dr, di = e[1][0] - e[3][0], e[1][1] - e[3][1]
    o0 = (ar + cr, ai + ci)
    o2 = (ar - cr, ai - ci)
    pm = (br - di, bi + dr)
    mm = (br + di, bi - dr)
    return [o0, pm, o2, mm] if sign > 0 else [o0, mm, o2, pm]


def _sel4(xt, lane4):
    odd = (lane4 & 1) == 1
    a = [[jnp.where(odd, xt[2 * r1 + 1], xt[2 * r1]) for r1 in range(2)],
         [jnp.where(odd, xt[2 * r1], xt[2 * r1 + 1]) for r1 in range(2)]]
    out = []
    for p in range(4):
        hi = ((lane4 - p) & 3) >= 2
        out.append(jnp.where(hi, a[p & 1][1], a[p & 1][0]))
    return out


def _cmul(k, u):
    return k[0] * u[0] - k[1] * u[1], k[0] * u[1] + k[1] * u[0]


def _pack(a, b):
    return pltpu.pack_elementwise([a, b], packed_dtype=bf16).astype(u32)


def _unpk(w, i):
    return pltpu.unpack_elementwise(w, index=i, packed_dtype=bf16, unpacked_dtype=f32)


class _Stats:
    def __init__(self):
        self.piv = None
        self.s1 = None
        self.s2 = None

    def add(self, x, use_pivot=True):
        if use_pivot:
            if self.piv is None:
                self.piv = jnp.broadcast_to(x[0:1, :], (8, x.shape[1]))
        for i in range(x.shape[0] // 8):
            d = x[8 * i:8 * (i + 1), :]
            if use_pivot:
                d = d - self.piv
            self.s1 = d if self.s1 is None else self.s1 + d
            self.s2 = d * d if self.s2 is None else self.s2 + d * d

    def finish(self):
        n = self.s1.shape[1]
        e1 = jnp.sum(self.s1, axis=0, keepdims=True) * (1.0 / D)
        e2 = jnp.sum(self.s2, axis=0, keepdims=True) * (1.0 / D)
        var = jnp.maximum(e2 - e1 * e1, 0.0)
        mean = e1 if self.piv is None else e1 + self.piv[0:1, :]
        rstd = jax.lax.rsqrt(var + EPS)
        return jnp.broadcast_to(mean, (8, n)), jnp.broadcast_to(rstd, (8, n))


def _rep(a, n):
    return jnp.concatenate([a] * n, axis=0)


def _kernel(q_hbm, k_hbm, v_hbm, sh_hbm, sk_hbm, sd_hbm, w1_hbm, b1_hbm, w2_hbm, b2_hbm,
            z_hbm, out_hbm,
            qb, kb, vb, skb, w1b, w1t, w2b, par, ebuf, hc0, hc1, hc2, vbuf, ybuf, halo,
            xn0, xn1, hres0, hres1, ob, sh_ref, sd_ref, b1_ref, b2_ref, fm_ref, gm_ref, z_ref,
            sems, fsem):
    xn = [xn0, xn1]
    hres = [hres0, hres1]
    hc = [hc0, hc1, hc2]

    copies = {}

    def add(name, src, dst):
        lst = copies.setdefault(name, [])
        lst.append(pltpu.make_async_copy(src, dst, sems.at[sum(len(v) for v in copies.values())]))

    def cols(ref, lo, n, rows=None):
        return ref.at[:, pl.ds(lo, n)] if rows is None else ref.at[pl.ds(rows[0], rows[1]), pl.ds(lo, n)]

    def add_conv(name, c, rows=None):
        for src, dst in ((k_hbm, kb), (v_hbm, vb), (sk_hbm, skb)):
            add(name, cols(src, c * B, B, rows), cols(dst, c * B, B, rows))

    def add_w(i):
        (a0, a1), (b0, b1) = WP[i]
        add('w%d' % i, cols(w1_hbm, a0 * FC, (a1 - a0) * FC), cols(w1b, a0 * FC, (a1 - a0) * FC, (0, D)))
        add('w%d' % i, cols(w2_hbm, b0 * FC, (b1 - b0) * FC), cols(w2b, b0 * FC, (b1 - b0) * FC))

    for src, dst in ((sh_hbm, sh_ref), (z_hbm, z_ref), (sd_hbm, sd_ref), (b2_hbm, b2_ref), (b1_hbm, b1_ref)):
        add('par', src, dst)
    add_conv('c0a', 0, (0, D // 2))
    add_conv('c0b', 0, (D // 2, D // 2))
    add('q0', cols(q_hbm, 0, B), cols(qb, 0, B))
    add_w(0)
    add_conv('c1', 1)
    for i in range(1, len(WP)):
        add_w(i)
    for c in range(1, NC):
        add('q%d' % c, cols(q_hbm, c * B, B), cols(qb, c * B, B))
        if c + 1 < NC:
            add_conv('c%d' % (c + 1), c + 1)
    for lst in copies.values():
        for cp in lst:
            cp.start()
    nin = sum(len(v) for v in copies.values())

    def wait(*names):
        with jax.named_scope("w_" + "_".join(names)):
            if not names:
                pltpu.semaphore_signal(fsem, 1)
                pltpu.semaphore_wait(fsem, 1)
            for nm in names:
                for cp in copies.pop(nm):
                    cp.wait()

    def out_copy(c):
        return pltpu.make_async_copy(cols(ob, c * B, B), cols(out_hbm, c * B, B), sems.at[nin + c])

    def make_fm(p):
        row = jax.lax.broadcasted_iota(jnp.int32, (64, 128), 0)
        g = (4 * jax.lax.broadcasted_iota(jnp.int32, (64, 128), 1) + 1).astype(f32)
        x = [_sample_index(2 * row + e, p).astype(f32) * g for e in range(2)]
        for z in range(2):
            fm_ref[p, :, 128 * z:128 * (z + 1)] = _pack(*[_cos2048(x[e] + 512.0 * z) for e in range(2)])

    def make_gm(p):
        row = jax.lax.broadcasted_iota(jnp.int32, (64, 128), 0)
        t = _sample_index(jax.lax.broadcasted_iota(jnp.int32, (64, 128), 1), p).astype(f32)
        x = [(4 * (2 * row + e) + 1).astype(f32) * t for e in range(2)]
        toks = []
        for z in range(2):
            w = _pack(*[_cos2048(x[e] + 512.0 * z) * (1.0 / B) for e in range(2)])
            gm_ref[p, 64 * z:64 * (z + 1), :] = w
            toks += [w[8 * i:8 * (i + 1), :] for i in range(8)]
        return toks

    wait()
    for p in range(R):
        make_fm(p)
    wait('par')
    zc = jnp.clip(z_ref[0], 0, 1)
    z8 = pl.multiple_of(8 * zc, 8)
    never = [jax.lax.broadcasted_iota(jnp.int32, (8, 128), 1) < z_ref[1 + i] for i in range(2)]

    def dview(ref):
        n = ref.shape[-2] - 8
        return ref.at[pl.ds(z8, n), :] if len(ref.shape) == 2 else ref.at[:, pl.ds(z8, n), :]

    ebuf_w, ybuf_w, vbuf_w = dview(ebuf), dview(ybuf), dview(vbuf)
    hc_w = [dview(a) for a in hc]
    xn_w = [dview(a) for a in xn]
    hres_w = [dview(a) for a in hres]
    w1b_w = w1b.at[pl.ds(pl.multiple_of(16 * zc, 16), KP), :]

    P = jnp.concatenate([sh_ref[...].astype(f32), sd_ref[...].astype(f32).reshape(1, D),
                         b2_ref[...].astype(f32).reshape(1, D), jnp.zeros((2, D), f32)], axis=0)
    Pp = jnp.concatenate([P, jnp.zeros((8, 64), f32)], axis=1)
    PT = jnp.concatenate([Pp] * 16, axis=0).T

    gtok = [w for p in range(R) for w in make_gm(p)]
    ptile = []
    for i in range(D // 8):
        w = PT[8 * i:8 * (i + 1), :]
        for q, t in enumerate(gtok[i * len(gtok) // (D // 8):(i + 1) * len(gtok) // (D // 8)]):
            w = jnp.where(never[q % 2], pltpu.bitcast(t, f32), w)
        ptile.append(w)
    plhs = jnp.concatenate(ptile, axis=0).astype(bf16)

    def set_par(j0, j1):
        n = 128 * (j1 - j0)
        onehot = (jax.lax.broadcasted_iota(jnp.int32, (128, n), 0)
                  == j0 + jax.lax.broadcasted_iota(jnp.int32, (128, n), 1) // 128)
        pb = jnp.dot(plhs, jnp.where(onehot, 1.0, 0.0).astype(bf16), preferred_element_type=f32)
        for j in range(j0, j1):
            par[j] = pb[:, 128 * (j - j0):128 * (j - j0 + 1)]

    set_par(0, 4)
    rowx = jax.lax.broadcasted_iota(jnp.int32, ((KP - D) // 2, B), 0)
    ones_rows = jnp.where(rowx == 0, jnp.uint32(0x3F80), jnp.uint32(0))
    for i in range(2):
        xn[i][D // 2:KP // 2, :] = ones_rows
    b1row = b1_ref[...].astype(f32).reshape(1, F)

    def prep_w(i):
        a0, a1 = WP[i][0]
        n = (a1 - a0) * FC
        row = jax.lax.broadcasted_iota(jnp.int32, (KP - D, n), 0)
        brow = jnp.broadcast_to(b1row[:, a0 * FC:a1 * FC], (KP - D, n))
        w1b_w[D:KP, a0 * FC:a1 * FC] = jnp.where(row == 0, brow, 0.0).astype(bf16)
        for j in range(a0, a1):
            w1t[j * FC // 2:(j + 1) * FC // 2, :] = pltpu.bitcast(w1b[0:KP, j * FC:(j + 1) * FC].T, u32)

    lane_w = jax.lax.broadcasted_iota(jnp.int32, (H, 128), 1)
    st = {}

    def slot(s):
        return slice(128 * s, 128 * (s + 1))

    def shuffle(blocks):
        xt = [blocks[0]] + [pltpu.roll(blocks[r], r, 1) for r in range(1, R)]
        return _sel4(xt, lane_w & 3)

    def stage_a(c, t):
        r0 = RT * t
        rows = slice(r0, r0 + RT)
        taps = [[par[s, pl.ds(r0 + e, H, stride=2), :] for s in range(4)] for e in range(2)]
        if c == 0:
            prev = [jnp.zeros((H, 128), u32)] * 3
        else:
            prev = [halo[H * t:H * (t + 1), slot(s)] for s in range(3)]
        sw = [pltpu.bitcast(skb[rows, c * B + 128 * r:c * B + 128 * (r + 1)], u32) for r in range(R)]
        pk = shuffle(sw)
        ub = []
        for r in range(R):
            ls = slice(c * B + 128 * r, c * B + 128 * (r + 1))
            kw = pltpu.bitcast(kb[rows, ls], u32)
            vw = pltpu.bitcast(vb[rows, ls], u32)
            cur = [pltpu.roll(kw, s, 1) for s in range(1, 4)]
            ks = [kw] + [jnp.where(lane_w >= s, cur[s - 1], prev[s - 1]) for s in range(1, 4)]
            prev = cur
            ue = []
            for e in range(2):
                acc = (_unpk(ks[0], e) * taps[e][0] + _unpk(ks[1], e) * taps[e][1]) + (
                    _unpk(ks[2], e) * taps[e][2] + _unpk(ks[3], e) * taps[e][3])
                ue.append(acc * _unpk(vw, e))
            ub.append(_pack(*ue))
        if c < NC - 1:
            for s in range(3):
                halo[H * t:H * (t + 1), slot(s)] = prev[s]
        return pk, shuffle(ub)

    def fwd(c, t0, nt):
        ops = [[] for _ in range(R)]
        for t in range(t0, t0 + nt):
            pk, pu = stage_a(c, t)
            for p in range(R):
                ops[p] += [pk[p], pu[p]]
        e = [None] * R
        for p in (0, 2, 1, 3):
            lhs = pltpu.bitcast(jnp.concatenate(ops[p], axis=0), bf16)
            e[p] = jnp.dot(lhs, pltpu.bitcast(fm_ref[p], bf16), preferred_element_type=f32)
        return e

    def stage_ab(c):
        t0 = 0
        for gr in GB:
            e = fwd(c, t0, gr // RT)
            for p in range(R):
                ebuf_w[2 * RT * t0:2 * RT * t0 + 2 * gr, 256 * p:256 * (p + 1)] = e[p]
            t0 += gr // RT

    def ld(ar, rows, s0):
        return [(ar[rows, slot(s0 + 2 * m)], ar[rows, slot(s0 + 2 * m + 1)]) for m in range(R)]

    def sto(ar, rows, s0, vals):
        for m in range(R):
            ar[rows, slot(s0 + 2 * m)] = vals[m][0]
            ar[rows, slot(s0 + 2 * m + 1)] = vals[m][1]

    def stage_c(c, t, e=None):
        toks = []
        vps = []
        for hf in range(2):
            r0 = RT * t + 8 * hf
            rows = slice(r0, r0 + 8)
            if e is None:
                eb = 2 * RT * t + 8 * hf
                ek, eu = ld(ebuf, slice(eb, eb + 8), 0), ld(ebuf, slice(eb + RT, eb + RT + 8), 0)
            else:
                ek, eu = [[(e[p][o:o + 8, 0:128], e[p][o:o + 8, 128:256]) for p in range(R)]
                          for o in (8 * hf, RT + 8 * hf)]
            km = _bfly(ek, -1)
            if c == 0:
                dd = par[4, rows, :]
                kc = [(km[m][0] + dd, km[m][1]) for m in range(R)]
            else:
                kprev = ld(hc[c - 1], rows, SR if c > 1 else SK)
                if c == 1:
                    dd = par[4, rows, :]
                    kprev = [(kprev[m][0] - dd, kprev[m][1]) for m in range(R)]
                kc = [(km[m][0] - kprev[m][1], km[m][1] + kprev[m][0]) for m in range(R)]
            um = _bfly(eu, -1)
            if c < NC - 1:
                ar = hc_w[c] if c > 0 else hc[0]
                if c > 0:
                    sto(ar, rows, SR, km)
                sto(ar, rows, SK, kc)
                sto(ar, rows, SU, um)
            ym = [None] * R
            for m in (0, 2, 1, 3):
                y = None
                for dl in range(c + 1):
                    k = kc[m] if dl == c else (hc[dl][rows, slot(SK + 2 * m)], hc[dl][rows, slot(SK + 2 * m + 1)])
                    u = um[m] if dl == 0 else (hc[c - dl][rows, slot(SU + 2 * m)], hc[c - dl][rows, slot(SU + 2 * m + 1)])
                    tt = _cmul(k, u)
                    y = tt if y is None else (y[0] + tt[0], y[1] + tt[1])
                ym[m] = y
                toks += [(y[0], 4 * (c + 1) + (14 if m < 2 else 6)), (y[1], 4 * (c + 1))]
            vps.append(_bfly(ym, +1))
        w = [[_pack(vps[0][p][z], vps[1][p][z]) for z in range(2)] for p in range(R)]
        if e is not None:
            return [jnp.concatenate(w[p], axis=1) for p in range(R)]
        for p in (0, 2, 1, 3):
            for z in range(2):
                vbuf_w[H * t:H * (t + 1), slot(2 * p + z)] = w[p][z]
                toks.append((w[p][z], 6))
        return toks

    def inv(v, t0, nt, dst):
        y = [jnp.dot(pltpu.bitcast(v[p], bf16), pltpu.bitcast(gm_ref[p], bf16), preferred_element_type=f32)
             for p in range(R)]
        for i in range(nt):
            yw = [_pack(y[p][RT * i:RT * i + 8, :], y[p][RT * i + 8:RT * (i + 1), :]) for p in range(R)]
            xt = _sel4(yw, lane_w & 3)
            for r in range(R):
                w = xt[r] if r == 0 else pltpu.roll(xt[r], 128 - r, 1)
                for e in range(2):
                    r0 = RT * (t0 + i) + 8 * e
                    dst[r, r0:r0 + 8, :] = _unpk(w, e)

    def stage_d(c):
        t0 = 0
        for gr in GD:
            nt = gr // RT
            inv([vbuf[H * t0:H * (t0 + nt), 256 * p:256 * (p + 1)] for p in range(R)], t0, nt, ybuf_w)
            t0 += nt

    def gate(a, i, on):
        return jnp.where(never[0], par[i // 56, 8 * (i % 56):8 * (i % 56) + 8, :], a) if on else a

    def stage_x(c, r):
        toks = []
        s = _Stats()
        for t in range(D // 32):
            s.add(qb[t * 32:(t + 1) * 32, c * B + 128 * r:c * B + 128 * (r + 1)].astype(f32))
            toks += [(s.s1, 13), (s.s2, 9)]
        st['xs', c, r] = s.finish()
        return toks

    def stage_e1(c, r, clk):
        hr = hres[c % 2]
        toks = []
        mx, rx = [_rep(a, 2) for a in st.pop(('xs', c, r))]
        s = _Stats()
        for t in range(NT):
            rows = slice(t * RT, (t + 1) * RT)
            x = qb[rows, c * B + 128 * r:c * B + 128 * (r + 1)].astype(f32)
            y = jnp.concatenate([ybuf[r, pl.ds(t * RT + e, H, stride=2), :] for e in range(2)], axis=0)
            h = x + (x - mx) * rx * y
            (hres_w[c % 2] if clk else hr)[r, rows, :] = h
            s.add(h)
            toks += [(s.s1, 15), (s.s2, 5)]
        st['hs', r] = s.finish()
        return toks

    def stage_e2(c, r, clk):
        hr = hres[c % 2]
        toks = []
        m1, r1 = st['hs', r]
        r1 = _rep(r1, 4)
        s = _Stats()
        for t in range(D // 32):
            m1g = _rep(gate(m1, 14 * r + t, clk), 4)
            s.add((hr[r, t * 32:(t + 1) * 32, :] - m1g) * r1, use_pivot=False)
            toks += [(s.s1, 14), (s.s2, 9)]
        st['ns', r] = s.finish()
        return toks

    def stage_e3(c, r, clk, gt=True):
        hr = hres[c % 2]
        toks = []
        (m1, r1), (m2, r2) = st.pop(('hs', r)), st.pop(('ns', r))
        for t in range(NT):
            if t % 2 == 0:
                m1g = gate(m1, 56 + 14 * r + t // 2, clk and gt)
            n2 = [((hr[r, pl.ds(t * RT + e, H, stride=2), :] - m1g) * r1 - m2) * r2 for e in range(2)]
            w = _pack(*n2)
            (xn_w if clk else xn)[c % 2][t * H:(t + 1) * H, slot(r)] = w
            toks.append((w, 10))
        return toks

    def hld(hr):
        return jnp.concatenate([hr[r, 0:D, :] for r in range(R)], axis=1)

    pts = {}

    def attach(w, key):
        for q, t in enumerate(pts.pop(key, ())):
            w = jnp.where(never[q % 2], pltpu.bitcast(t, u32), w)
        return w

    def mm1(c, j):
        if any(k[:3] == (c, 1, j) for k in pts):
            zs = []
            for n in range(R):
                tiles = []
                for i in range(FC // RT):
                    w = w1t[j * FC // 2 + H * i:j * FC // 2 + H * (i + 1), :]
                    if (c, 1, j, n, i) in pts:
                        w = jnp.concatenate([attach(w[:, 0:128], (c, 1, j, n, i)), w[:, 128:]], axis=1)
                    tiles.append(w)
                lhs = pltpu.bitcast(jnp.concatenate(tiles, axis=0), bf16)
                zs.append(jnp.dot(lhs, pltpu.bitcast(xn[c % 2][0:KP // 2, slot(n)], bf16),
                                  preferred_element_type=f32))
            z = jnp.concatenate(zs, axis=1)
        else:
            lhs = pltpu.bitcast(w1t[j * FC // 2:(j + 1) * FC // 2, :], bf16)
            z = jnp.dot(lhs, pltpu.bitcast(xn[c % 2][0:KP // 2, :], bf16), preferred_element_type=f32)
        t = jnp.tanh(z * (C1 + C2 * (z * z)))
        hz = 0.5 * z
        st['ht', j] = (hz + hz * t).astype(bf16)

    def mm2(c, j):
        lhs = w2b[:, j * FC:(j + 1) * FC]
        if any((c, 2, j, i) in pts for i in range(NT)):
            tiles = [attach(pltpu.bitcast(lhs[RT * i:RT * (i + 1), :], u32), (c, 2, j, i)) for i in range(NT)]
            lhs = pltpu.bitcast(jnp.concatenate(tiles, axis=0), bf16)
        acc = hld(hres[c % 2]) + jnp.dot(lhs, st.pop(('ht', j)), preferred_element_type=f32)
        if j < NF - 1:
            for r in range(R):
                hres[c % 2][r, 0:D, :] = acc[:, slot(r)]
        else:
            acc = acc + jnp.concatenate([par[5]] * R, axis=1)
            ob[:, pl.ds(c * B, B)] = acc.astype(bf16)
            out_copy(c).start()

    seq = [(1, 0)] + [x for j in range(NF) for x in ([(1, j + 1)] if j + 1 < NF else []) + [(2, j)]]

    def points(c, i0, i1):
        out = []
        for kind, j in seq[i0:i1]:
            if kind == 1:
                out += [(c, 1, j, n, i) for n in range(R) for i in range(FC // RT)]
            else:
                out += [(c, 2, j, i) for i in range(NT)]
        return out

    def place(toks, keys):
        total = sum(w for _, w in toks)
        acc = 0
        for t, w in toks:
            acc += w
            k = min(len(keys) - 1, (acc * len(keys) - 1) // total)
            pts.setdefault(keys[k], []).append(t)

    go = [sum(G0[:g]) // RT for g in range(len(G0))]

    def c0_ab(g):
        st['e', g] = fwd(0, go[g], G0[g] // RT)

    def c0_cd(g):
        e = st.pop(('e', g))
        v = [stage_c(0, go[g] + i, [x[2 * RT * i:2 * RT * (i + 1), :] for x in e]) for i in range(G0[g] // RT)]
        inv([jnp.concatenate([w[p] for w in v], axis=0) for p in range(R)], go[g], G0[g] // RT, ybuf)

    wait('c0a')
    set_par(4, 6)
    for ev in ORDER0.split():
        if ev == '|':
            wait('c0b')
        else:
            (c0_ab if ev[0] == 'a' else c0_cd)(int(ev[1]))
    wait('q0', 'w0')
    prep_w(0)
    for r in range(R):
        stage_x(0, r)
        stage_e1(0, r, False)
        stage_e2(0, r, False)
        stage_e3(0, r, False)
    fence_ab = [None, ('w2',), ('q2', 'c3'), ('q3',)]
    for c in range(NC):
        n = c + 1
        for i, (kind, j) in enumerate(seq):
            if c == 0 and i == POS_C1:
                wait('c1', 'w1')
                prep_w(1)
            if n < NC and i == POS_AB[c]:
                stage_ab(n)
            if n < NC and i == POS_FAB[c]:
                wait(*fence_ab[n])
                if c == 0:
                    prep_w(2)
                toks = []
                for t in range(NT):
                    toks += stage_c(n, t)
                    if t % 7 == 3 and n > 1:
                        toks += stage_x(n, t // 7)
                place(toks, points(c, i, POS_D[c])[6:-4])
            if n < NC and i == POS_D[c]:
                stage_d(n)
                if n > 1:
                    for r in range(R):
                        stage_e1(n, r, True)
                    for r in range(R):
                        stage_e2(n, r, False)
                    for r in range(R):
                        stage_e3(n, r, True, False)
            if c == 0 and i == POS_FD:
                wait('w3', 'q1', 'c2')
                prep_w(3)
                keys = points(c, i, len(seq) - 1)
                b = [int(len(keys) * x) for x in [0.0, 0.2, 0.56, 0.78, 1.0]]
                place([x for r in range(R) for x in stage_x(n, r)], keys[6:b[1]])
                place([x for r in range(R) for x in stage_e1(n, r, True)], keys[b[1] + 6:b[2]])
                place([x for r in range(R) for x in stage_e2(n, r, True)], keys[b[2] + 8:b[3]])
                place([x for r in range(R) for x in stage_e3(n, r, True)], keys[b[3] + 8:b[4]])
            (mm1 if kind == 1 else mm2)(c, j)
    for c in range(NC):
        out_copy(c).wait()


@jax.jit
def pallas_sequential_preLN__ssm_conv_h3__mixer_channel_mlp__prompt_kernel(
        A_q, A_k, A_v, A_shift_k, A_ssm_k, A_ssm_D, B_x, B_w1, B_b1, B_w2, B_b2):
    qT, kT, vT = A_q[0].T, A_k[0].T, A_v[0].T
    anyspec = pl.BlockSpec(memory_space=pl.ANY)
    out = pl.pallas_call(
        _kernel,
        out_shape=jax.ShapeDtypeStruct((D, S), bf16),
        in_specs=[anyspec] * 11,
        out_specs=anyspec,
        scratch_shapes=[
            pltpu.VMEM((D, S), bf16), pltpu.VMEM((D, S), bf16), pltpu.VMEM((D, S), bf16), pltpu.VMEM((D, S), bf16),
            pltpu.VMEM((KP + 16, F), bf16), pltpu.VMEM((F // 2, KP), u32), pltpu.VMEM((D, F), bf16),
            pltpu.VMEM((6, D, 128), f32),
            pltpu.VMEM((2 * D + 8, 2 * B), f32),
            *[pltpu.VMEM((D + 8, HL), f32)] * (NC - 1),
            pltpu.VMEM((D // 2 + 8, 2 * B), u32), pltpu.VMEM((R, D + 8, 128), f32), pltpu.VMEM((D // 2, 384), u32),
            pltpu.VMEM((KP // 2 + 8, B), u32), pltpu.VMEM((KP // 2 + 8, B), u32),
            pltpu.VMEM((R, D + 8, 128), f32), pltpu.VMEM((R, D + 8, 128), f32),
            pltpu.VMEM((D, S), bf16),
            pltpu.VMEM((4, D), bf16), pltpu.VMEM((D,), bf16), pltpu.VMEM((F,), bf16), pltpu.VMEM((D,), bf16),
            pltpu.VMEM((R, 64, 256), u32), pltpu.VMEM((R, 128, 128), u32), pltpu.SMEM((3,), jnp.int32),
            pltpu.SemaphoreType.DMA((40,)), pltpu.SemaphoreType.REGULAR,
        ],
        compiler_params=pltpu.CompilerParams(vmem_limit_bytes=100 * 1024 * 1024),
    )(qT, kT, vT, A_shift_k.T, A_ssm_k, A_ssm_D, B_w1, B_b1, B_w2.T, B_b2, np.zeros((3,), np.int32))
    return out.T[None]
```

```python
import jax
import jax.numpy as jnp
import jax.experimental.pallas as pl
import jax.experimental.pallas.tpu as pltpu

S, D, F = 2048, 448, 1792
B = 512
R = 4
NC = S // B
KP = 512
FC = 128
NF = F // FC
RT = 16
NT = D // RT
H = RT // 2
GB = [112] * 4
GD = [112] * 4
G0 = [64, 64, 48, 48, 64, 64, 48, 48]
ORDER0 = 'a0 a1 c0 a2 c1 a3 | c2 a4 c3 a5 c4 a6 c5 a7 c6 c7'
OG = 4
PAD = 200
EPS = 1e-5
f32 = jnp.float32
bf16 = jnp.bfloat16
u32 = jnp.uint32
C1 = 0.7978845608028654
C2 = C1 * 0.044715
SK, SU = 0, 8
HL = 17 * 128
POS_W1 = 6
POS_C1 = 11
POS_AB = [13, 3, 3]
POS_FAB = [13, 3, 3]
POS_D = [20, 21, 21]
POS_FD = 21
WP = [((0, 4), (0, 2)), ((4, 8), (2, 7)), ((8, 11), (7, 7)), ((11, 14), (7, 14))]


def _cos2048(x):
    n = x - 2048.0 * jnp.floor(x * (1.0 / 2048.0))
    u = jnp.abs(n - 1024.0) * (1.0 / 512.0) - 1.0
    u2 = u * u
    pl_ = 1.6044118478735982e-04
    for cf in (-4.681754135318688e-03, 7.969262624616703e-02, -6.459640975062462e-01, 1.5707963267948966):
        pl_ = pl_ * u2 + cf
    return pl_ * u


def _sample_index(b, p):
    r = (b - p) & 3
    return 128 * r + ((b - r) & 127)


def _bfly(e, sign):
    ar, ai = e[0][0] + e[2][0], e[0][1] + e[2][1]
    br, bi = e[0][0] - e[2][0], e[0][1] - e[2][1]
    cr, ci = e[1][0] + e[3][0], e[1][1] + e[3][1]
    dr, di = e[1][0] - e[3][0], e[1][1] - e[3][1]
    o0 = (ar + cr, ai + ci)
    o2 = (ar - cr, ai - ci)
    pm = (br - di, bi + dr)
    mm = (br + di, bi - dr)
    return [o0, pm, o2, mm] if sign > 0 else [o0, mm, o2, pm]


def _sel4(xt, lane4):
    odd = (lane4 & 1) == 1
    a = [[jnp.where(odd, xt[2 * r1 + 1], xt[2 * r1]) for r1 in range(2)],
         [jnp.where(odd, xt[2 * r1], xt[2 * r1 + 1]) for r1 in range(2)]]
    out = []
    for p in range(4):
        hi = ((lane4 - p) & 3) >= 2
        out.append(jnp.where(hi, a[p & 1][1], a[p & 1][0]))
    return out


def _cmul(k, u):
    return k[0] * u[0] - k[1] * u[1], k[0] * u[1] + k[1] * u[0]


def _pack(x):
    return pltpu.bitcast(x.astype(bf16), u32)


def _unpk(w):
    return pltpu.bitcast(w, bf16).astype(f32)


class _Stats:
    def __init__(self):
        self.piv = None
        self.s1 = None
        self.s2 = None

    def add(self, x, use_pivot=True):
        if use_pivot:
            if self.piv is None:
                self.piv = jnp.broadcast_to(x[0:1, :], (8, x.shape[1]))
        for i in range(x.shape[0] // 8):
            d = x[8 * i:8 * (i + 1), :]
            if use_pivot:
                d = d - self.piv
            self.s1 = d if self.s1 is None else self.s1 + d
            self.s2 = d * d if self.s2 is None else self.s2 + d * d

    def finish(self):
        n = self.s1.shape[1]
        e1 = jnp.sum(self.s1, axis=0, keepdims=True) * (1.0 / D)
        e2 = jnp.sum(self.s2, axis=0, keepdims=True) * (1.0 / D)
        var = jnp.maximum(e2 - e1 * e1, 0.0)
        mean = e1 if self.piv is None else e1 + self.piv[0:1, :]
        rstd = jax.lax.rsqrt(var + EPS)
        return jnp.broadcast_to(mean, (8, n)), jnp.broadcast_to(rstd, (8, n))


def _rep(a, n):
    return jnp.concatenate([a] * n, axis=0)


def _kernel(q_hbm, k_hbm, v_hbm, sh_hbm, sk_hbm, sd_hbm, w1_hbm, b1_hbm, w2_hbm, b2_hbm,
            out_hbm,
            qb, kb, vb, skb, w1b, w1t, w2b, par, ebuf, hc0, hc1, hc2, vbuf, ybuf, halo,
            xn0, xn1, hres0, hres1, ob, sh_ref, sd_ref, b1_ref, b2_ref, fm_ref, gm_ref,
            sems, fsem):
    xn = [xn0, xn1]
    hres = [hres0, hres1]
    hc = [hc0, hc1, hc2]

    copies = {}

    def add(name, src, dst):
        lst = copies.setdefault(name, [])
        lst.append(pltpu.make_async_copy(src, dst, sems.at[sum(len(v) for v in copies.values())]))

    def cols(ref, lo, n, rows=None):
        return ref.at[:, pl.ds(lo, n)] if rows is None else ref.at[pl.ds(rows[0], rows[1]), pl.ds(lo, n)]

    def add_conv(name, c, rows=None):
        for src, dst in ((k_hbm, kb), (v_hbm, vb), (sk_hbm, skb)):
            add(name, cols(src, c * B, B, rows), cols(dst, c * B, B, rows))

    def add_w(i):
        (a0, a1), (b0, b1) = WP[i]
        add('w%d' % i, cols(w1_hbm, a0 * FC, (a1 - a0) * FC), cols(w1b, a0 * FC, (a1 - a0) * FC, (0, D)))
        if b1 > b0:
            add('w%d' % i, cols(w2_hbm, b0 * FC, (b1 - b0) * FC), cols(w2b, b0 * FC, (b1 - b0) * FC))

    for src, dst in ((sh_hbm, sh_ref), (sd_hbm, sd_ref), (b2_hbm, b2_ref), (b1_hbm, b1_ref)):
        add('par', src, dst)
    add_conv('c0a', 0, (0, D // 2))
    add_conv('c0b', 0, (D // 2, D // 2))
    add('q0', cols(q_hbm, 0, B), cols(qb, 0, B))
    add_w(0)
    add_w(1)
    add_conv('c1', 1)
    add_w(2)
    add_w(3)
    for c in range(1, NC):
        add('q%d' % c, cols(q_hbm, c * B, B), cols(qb, c * B, B))
        if c + 1 < NC:
            add_conv('c%d' % (c + 1), c + 1)
    for lst in copies.values():
        for cp in lst:
            cp.start()
    nin = sum(len(v) for v in copies.values())

    def wait(*names):
        if not names:
            pl.semaphore_signal(fsem, 1)
            pl.semaphore_wait(fsem, 1)
        for nm in names:
            for cp in copies.pop(nm):
                cp.wait()

    def out_copies(c):
        if c < NC - 1:
            blks = [(0, D, c * B, B)]
        else:
            gr = D // OG
            blks = [(0, D, c * B, B // 2)] + [(g * gr, gr, c * B + B // 2, B // 2) for g in range(OG)]
        return [(b, pltpu.make_async_copy(cols(ob, b[2], b[3], b[:2]), cols(out_hbm, b[2], b[3], b[:2]),
                                          sems.at[nin + c + g])) for g, b in enumerate(blks)]

    def make_fm(p):
        t = _sample_index(jax.lax.broadcasted_iota(jnp.int32, (128, 128), 0), p).astype(f32)
        x = t * (4 * jax.lax.broadcasted_iota(jnp.int32, (128, 128), 1) + 1).astype(f32)
        for z in range(2):
            fm_ref[p, :, 128 * z:128 * (z + 1)] = _pack(_cos2048(x + 512.0 * z))

    def make_gm(p):
        t = _sample_index(jax.lax.broadcasted_iota(jnp.int32, (128, 128), 1), p).astype(f32)
        x = t * (4 * jax.lax.broadcasted_iota(jnp.int32, (128, 128), 0) + 1).astype(f32)
        toks = []
        for z in range(2):
            w = _pack(_cos2048(x + 512.0 * z) * (1.0 / B))
            gm_ref[p, 64 * z:64 * (z + 1), :] = w
            toks += [w[8 * i:8 * (i + 1), :] for i in range(8)]
        return toks

    wait()
    for p in range(R):
        make_fm(p)
    wait('par')
    i0 = jax.lax.broadcasted_iota(jnp.int32, (8, 128), 0)
    i1 = jax.lax.broadcasted_iota(jnp.int32, (8, 128), 1)
    zero = [jnp.min(a.astype(f32)).astype(jnp.int32) for a in (i0 + i1, i1, 2 * i1 + i0)]
    z8 = pl.multiple_of(jnp.clip(8 * zero[0], 0, 8), 8)
    never = [i1 < zero[1 + i] for i in range(2)]

    def dview(ref):
        n = ref.shape[-2] - 8
        return ref.at[pl.ds(z8, n), :] if len(ref.shape) == 2 else ref.at[:, pl.ds(z8, n), :]

    ybuf_w = dview(ybuf)
    xn_w = [dview(a) for a in xn]
    hres_w = [dview(a) for a in hres]

    P = jnp.concatenate([sh_ref[...].astype(f32), sd_ref[...].astype(f32).reshape(1, D),
                         b2_ref[...].astype(f32).reshape(1, D), jnp.zeros((2, D), f32)], axis=0)
    Pp = jnp.concatenate([P, jnp.zeros((8, 64), f32)], axis=1)
    PT = jnp.concatenate([Pp] * 16, axis=0).T

    gtok = [w for p in range(R) for w in make_gm(p)]
    ptile = []
    for i in range(D // 8):
        w = PT[8 * i:8 * (i + 1), :]
        for q, t in enumerate(gtok[i * len(gtok) // (D // 8):(i + 1) * len(gtok) // (D // 8)]):
            w = jnp.where(never[q % 2], pltpu.bitcast(t, f32), w)
        ptile.append(w)
    plhs = jnp.concatenate(ptile, axis=0).astype(bf16)

    def set_par(j0, j1):
        n = 128 * (j1 - j0)
        onehot = (jax.lax.broadcasted_iota(jnp.int32, (128, n), 0)
                  == j0 + jax.lax.broadcasted_iota(jnp.int32, (128, n), 1) // 128)
        pb = jnp.dot(plhs, jnp.where(onehot, 1.0, 0.0).astype(bf16), preferred_element_type=f32)
        for j in range(j0, j1):
            par[j] = pb[:, 128 * (j - j0):128 * (j - j0 + 1)]

    set_par(0, 4)
    rowx = jax.lax.broadcasted_iota(jnp.int32, ((KP - D) // 2, B), 0)
    ones_rows = jnp.where(rowx == 0, jnp.uint32(0x3F80), jnp.uint32(0))
    for i in range(2):
        xn[i][D // 2:KP // 2, :] = ones_rows
    b1row = b1_ref[...].astype(f32).reshape(1, F)

    row = jax.lax.broadcasted_iota(jnp.int32, (KP - D, F), 0)
    w1b[D:KP, :] = jnp.where(row == 0, jnp.broadcast_to(b1row, (KP - D, F)), 0.0).astype(bf16)

    def prep_w(i):
        a0, a1 = WP[i][0]
        for j in range(a0, a1):
            w1t[j * FC // 2:(j + 1) * FC // 2, :] = pltpu.bitcast(w1b[0:KP, j * FC:(j + 1) * FC].T, u32)

    lane_w = jax.lax.broadcasted_iota(jnp.int32, (H, 128), 1)
    lane_t = jax.lax.broadcasted_iota(jnp.int32, (RT, 128), 1)
    st = {}

    def slot(s):
        return slice(128 * s, 128 * (s + 1))

    def shuffle(blocks):
        xt = [blocks[0]] + [pltpu.roll(blocks[r], r, 1) for r in range(1, R)]
        return _sel4(xt, lane_w & 3)

    def stage_a(c, t):
        r0 = RT * t
        rows = slice(r0, r0 + RT)
        taps = [par[s, rows, :] for s in range(4)]
        if c == 0:
            prev = [jnp.zeros((H, 128), u32)] * 3
        else:
            prev = [halo[H * t:H * (t + 1), slot(s)] for s in range(3)]
        sw = [pltpu.bitcast(skb[rows, c * B + 128 * r:c * B + 128 * (r + 1)], u32) for r in range(R)]
        pk = shuffle(sw)
        ub = []
        for r in range(R):
            ls = slice(c * B + 128 * r, c * B + 128 * (r + 1))
            kw = pltpu.bitcast(kb[rows, ls], u32)
            cur = [pltpu.roll(kw, s, 1) for s in range(1, 4)]
            ks = [kw] + [jnp.where(lane_w >= s, cur[s - 1], prev[s - 1]) for s in range(1, 4)]
            prev = cur
            acc = (_unpk(ks[0]) * taps[0] + _unpk(ks[1]) * taps[1]) + (
                _unpk(ks[2]) * taps[2] + _unpk(ks[3]) * taps[3])
            ub.append(_pack(acc * vb[rows, ls].astype(f32)))
        if c < NC - 1:
            for s in range(3):
                halo[H * t:H * (t + 1), slot(s)] = prev[s]
        return pk, shuffle(ub)

    def fwd(c, t0, nt):
        ops = [[] for _ in range(R)]
        for t in range(t0, t0 + nt):
            pk, pu = stage_a(c, t)
            for p in range(R):
                ops[p] += [pk[p], pu[p]]
        e = [None] * R
        for p in (0, 2, 1, 3):
            lhs = pltpu.bitcast(jnp.concatenate(ops[p], axis=0), bf16)
            e[p] = jnp.dot(lhs, pltpu.bitcast(fm_ref[p], bf16), preferred_element_type=f32)
        return e

    def stage_ab(c):
        t0 = 0
        for gr in GB:
            e = fwd(c, t0, gr // RT)
            for p in range(R):
                ebuf[2 * RT * t0:2 * RT * t0 + 2 * gr, 256 * p:256 * (p + 1)] = e[p]
            t0 += gr // RT

    def ld(ar, rows, s0):
        return [(ar[rows, slot(s0 + 2 * m)], ar[rows, slot(s0 + 2 * m + 1)]) for m in range(R)]

    def sto(ar, rows, s0, vals):
        for m in range(R):
            ar[rows, slot(s0 + 2 * m)] = vals[m][0]
            ar[rows, slot(s0 + 2 * m + 1)] = vals[m][1]

    def stage_c(c, t, e=None):
        toks = []
        vps = []
        for hf in range(2):
            r0 = RT * t + 8 * hf
            rows = slice(r0, r0 + 8)
            if e is None:
                eb = 2 * RT * t + 8 * hf
                ek, eu = ld(ebuf, slice(eb, eb + 8), 0), ld(ebuf, slice(eb + RT, eb + RT + 8), 0)
            else:
                ek, eu = [[(e[p][o:o + 8, 0:128], e[p][o:o + 8, 128:256]) for p in range(R)]
                          for o in (8 * hf, RT + 8 * hf)]
            km = _bfly(ek, -1)
            if c == 0:
                dd = par[4, rows, :]
                kc = [(km[m][0] + dd, km[m][1]) for m in range(R)]
            else:
                dd = par[4, rows, :]
                kprev = [(a - dd, b) for a, b in ld(hc[0], rows, SK)]
                for cc in range(1, c):
                    kq = ld(hc[cc], rows, SK)
                    kprev = [(kq[m][0] + kprev[m][1], kq[m][1] - kprev[m][0]) for m in range(R)]
                kc = [(km[m][0] - kprev[m][1], km[m][1] + kprev[m][0]) for m in range(R)]
            um = _bfly(eu, -1)
            if c < NC - 1:
                sto(hc[c], rows, SK, kc)
                sto(hc[c], rows, SU, um)
            ym = [None] * R
            for m in (0, 2, 1, 3):
                y = None
                for dl in range(c + 1):
                    k = kc[m] if dl == c else (hc[dl][rows, slot(SK + 2 * m)], hc[dl][rows, slot(SK + 2 * m + 1)])
                    u = um[m] if dl == 0 else (hc[c - dl][rows, slot(SU + 2 * m)], hc[c - dl][rows, slot(SU + 2 * m + 1)])
                    tt = _cmul(k, u)
                    y = tt if y is None else (y[0] + tt[0], y[1] + tt[1])
                ym[m] = y
                toks += [(y[0], 6 * c + 3 + (14 if m < 2 else 6)), (y[1], 4 * (c + 1))]
            vp = _bfly(ym, +1)
            vps.append(vp)
            if e is None:
                sto(vbuf, rows, 0, vp)
                toks += [(vp[p][z], 3) for p in (0, 2, 1, 3) for z in range(2)]
        if e is None:
            return toks
        return [jnp.concatenate([jnp.concatenate(vps[hf][p], axis=1) for hf in range(2)], axis=0)
                for p in range(R)]

    def inv(v, t0, nt, dst):
        y = [jnp.dot(v[p].astype(bf16), pltpu.bitcast(gm_ref[p], bf16), preferred_element_type=f32)
             for p in range(R)]
        for i in range(nt):
            xt = _sel4([y[p][RT * i:RT * (i + 1), :] for p in range(R)], lane_t & 3)
            for r in range(R):
                dst[r, RT * (t0 + i):RT * (t0 + i + 1), :] = xt[r] if r == 0 else pltpu.roll(xt[r], 128 - r, 1)

    def stage_d(c):
        t0 = 0
        for gr in GD:
            nt = gr // RT
            inv([vbuf[RT * t0:RT * (t0 + nt), 256 * p:256 * (p + 1)] for p in range(R)], t0, nt,
                ybuf_w if c > 1 else ybuf)
            t0 += nt

    def gate(a, i, on):
        return jnp.where(never[0], par[i // 56, 8 * (i % 56):8 * (i % 56) + 8, :], a) if on else a

    def stage_x(c, r):
        toks = []
        s = _Stats()
        for t in range(D // 32):
            s.add(qb[t * 32:(t + 1) * 32, c * B + 128 * r:c * B + 128 * (r + 1)].astype(f32))
            toks += [(s.s1, 13), (s.s2, 9)]
        st['xs', c, r] = s.finish()
        return toks

    def stage_e1(c, r, clk):
        hr = hres[c % 2]
        toks = []
        mx, rx = [_rep(a, 2) for a in st.pop(('xs', c, r))]
        s = _Stats()
        for t in range(NT):
            rows = slice(t * RT, (t + 1) * RT)
            x = qb[rows, c * B + 128 * r:c * B + 128 * (r + 1)].astype(f32)
            y = ybuf[r, rows, :]
            h = x + (x - mx) * rx * y
            (hres_w[c % 2] if c > 1 else hr)[r, rows, :] = h
            s.add(h)
            toks += [(s.s1, 15), (s.s2, 5)]
        st['hs', r] = s.finish()
        return toks

    def stage_e2(c, r, clk):
        hr = hres[c % 2]
        toks = []
        m1, r1 = st['hs', r]
        r1 = _rep(r1, 4)
        s = _Stats()
        for t in range(D // 32):
            m1g = _rep(gate(m1, 14 * r + t, clk), 4)
            s.add((hr[r, t * 32:(t + 1) * 32, :] - m1g) * r1, use_pivot=False)
            toks += [(s.s1, 14), (s.s2, 9)]
        st['ns', r] = s.finish()
        return toks

    def stage_e3(c, r, clk, gt=True):
        hr = hres[c % 2]
        toks = []
        (m1, r1), (m2, r2) = st.pop(('hs', r)), st.pop(('ns', r))
        r1, m2, r2 = _rep(r1, 2), _rep(m2, 2), _rep(r2, 2)
        for t in range(NT):
            if t % 2 == 0:
                m1g = _rep(gate(m1, 56 + 14 * r + t // 2, clk and gt), 2)
            w = _pack(((hr[r, t * RT:(t + 1) * RT, :] - m1g) * r1 - m2) * r2)
            (xn_w if c > 1 else xn)[c % 2][t * H:(t + 1) * H, slot(r)] = w
            toks.append((w, 14))
        return toks

    def hld(hr):
        return jnp.concatenate([hr[r, 0:D, :] for r in range(R)], axis=1)

    pts = {}

    def attach(w, key):
        for q, t in enumerate(pts.pop(key, ())):
            w = jnp.where(never[q % 2], pltpu.bitcast(t, u32), w)
        return w

    def mm1(c, j):
        if any(k[:3] == (c, 1, j) for k in pts):
            zs = []
            for n in range(R):
                tiles = []
                for i in range(FC // RT):
                    w = w1t[j * FC // 2 + H * i:j * FC // 2 + H * (i + 1), :]
                    if (c, 1, j, n, i) in pts:
                        w = jnp.concatenate([attach(w[:, 0:128], (c, 1, j, n, i)), w[:, 128:]], axis=1)
                    tiles.append(w)
                lhs = pltpu.bitcast(jnp.concatenate(tiles, axis=0), bf16)
                zs.append(jnp.dot(lhs, pltpu.bitcast(xn[c % 2][0:KP // 2, slot(n)], bf16),
                                  preferred_element_type=f32))
            z = jnp.concatenate(zs, axis=1)
        else:
            lhs = pltpu.bitcast(w1t[j * FC // 2:(j + 1) * FC // 2, :], bf16)
            z = jnp.dot(lhs, pltpu.bitcast(xn[c % 2][0:KP // 2, :], bf16), preferred_element_type=f32)
        gelu(z, j)

    def gelu(z, j):
        t = jnp.tanh(z * (C1 + C2 * (z * z)))
        hz = 0.5 * z
        st['ht', j] = (hz + hz * t).astype(bf16)

    def mm1_first(c, nj):
        lhs = pltpu.bitcast(w1t[0:nj * FC // 2, :], bf16)
        z = jnp.dot(lhs, pltpu.bitcast(xn[c % 2][0:KP // 2, :], bf16), preferred_element_type=f32)
        for j in range(nj):
            gelu(z[j * FC:(j + 1) * FC, :], j)

    def mm2(c, j):
        lhs = w2b[:, j * FC:(j + 1) * FC]
        if any((c, 2, j, i) in pts for i in range(NT)):
            tiles = [attach(pltpu.bitcast(lhs[RT * i:RT * (i + 1), :], u32), (c, 2, j, i)) for i in range(NT)]
            lhs = pltpu.bitcast(jnp.concatenate(tiles, axis=0), bf16)
        acc = hld(hres[c % 2]) + jnp.dot(lhs, st.pop(('ht', j)), preferred_element_type=f32)
        if j < NF - 1:
            for r in range(R):
                hres[c % 2][r, 0:D, :] = acc[:, slot(r)]
        else:
            acc = acc + jnp.concatenate([par[5]] * R, axis=1)
            ob[:, pl.ds(c * B, B)] = acc.astype(bf16)
            out_copies(c)[0][1].start()

    def mm2_last(c):
        ht = jnp.concatenate([st.pop(('ht', NF - 2)), st.pop(('ht', NF - 1))], axis=0)
        cps = out_copies(c)
        for hf in range(2):
            acc = jnp.concatenate([hres[c % 2][2 * hf + r, 0:D, :] + par[5] for r in range(2)], axis=1)
            acc = acc + jnp.dot(w2b[:, (NF - 2) * FC:], ht[:, hf * B // 2:(hf + 1) * B // 2],
                                preferred_element_type=f32)
            for (r0, nr, c0, ncol), cp in (cps[:1] if hf == 0 else cps[1:]):
                ob[r0:r0 + nr, c0:c0 + ncol] = acc[r0:r0 + nr, :].astype(bf16)
                cp.start()

    seq = [(1, 0)] + [x for j in range(NF) for x in ([(1, j + 1)] if j + 1 < NF else []) + [(2, j)]]

    def points(c, i0, i1):
        out = []
        for kind, j in seq[i0:i1]:
            if kind == 1:
                out += [(c, 1, j, n, i) for n in range(R) for i in range(FC // RT)]
            else:
                out += [(c, 2, j, i) for i in range(NT)]
        return out

    def place(toks, keys):
        total = sum(w for _, w in toks)
        acc = 0
        for t, w in toks:
            acc += w
            k = min(len(keys) - 1, (acc * len(keys) - 1) // total)
            pts.setdefault(keys[k], []).append(t)

    go = [sum(G0[:g]) // RT for g in range(len(G0))]

    def c0_ab(g):
        st['e', g] = fwd(0, go[g], G0[g] // RT)

    def c0_cd(g):
        e = st.pop(('e', g))
        v = [stage_c(0, go[g] + i, [x[2 * RT * i:2 * RT * (i + 1), :] for x in e]) for i in range(G0[g] // RT)]
        inv([jnp.concatenate([w[p] for w in v], axis=0) for p in range(R)], go[g], G0[g] // RT, ybuf)

    wait('c0a')
    set_par(4, 6)
    for ev in ORDER0.split():
        if ev == '|':
            wait('c0b')
        else:
            (c0_ab if ev[0] == 'a' else c0_cd)(int(ev[1]))
    wait('q0', 'w0')
    prep_w(0)
    for r in range(R):
        stage_x(0, r)
        stage_e1(0, r, False)
        stage_e2(0, r, False)
        stage_e3(0, r, False)
    fence_ab = [None, ('w3',), ('q2', 'c3'), ('q3',)]
    for c in range(NC):
        n = c + 1
        for i, (kind, j) in enumerate(seq):
            if c == 0 and i == POS_W1:
                wait('w1')
                prep_w(1)
            if c == 0 and i == POS_C1:
                wait('c1', 'w2')
                prep_w(2)
            if n < NC and i == POS_AB[c]:
                stage_ab(n)
            if n < NC and i == POS_FAB[c]:
                wait(*fence_ab[n])
                if c == 0:
                    prep_w(3)
                toks = []
                for t in range(NT):
                    toks += stage_c(n, t)
                    if t % 7 == 3 and n > 1:
                        toks += stage_x(n, t // 7)
                place(toks, points(c, i, POS_D[c])[6:-4])
            if n < NC and i == POS_D[c]:
                stage_d(n)
                if n > 1:
                    for r in range(R):
                        stage_e1(n, r, True)
                    for r in range(R):
                        stage_e2(n, r, False)
                    for r in range(R):
                        stage_e3(n, r, True, False)
            if c == 0 and i == POS_FD:
                wait('q1', 'c2')
                keys = points(c, i, len(seq) - 1)
                b = [int(len(keys) * x) for x in [0.0, 0.2, 0.56, 0.78, 1.0]]
                place([x for r in range(R) for x in stage_x(n, r)], keys[6:b[1]])
                place([x for r in range(R) for x in stage_e1(n, r, True)], keys[b[1] + 6:b[2]])
                place([x for r in range(R) for x in stage_e2(n, r, True)], keys[b[2] + 8:b[3]])
                place([x for r in range(R) for x in stage_e3(n, r, True)], keys[b[3] + 8:b[4]])
            if c == 0 and kind == 1 and j < 4:
                if j == 0:
                    mm1_first(0, 4)
            elif c == NC - 1 and kind == 2 and j >= NF - 2:
                if j == NF - 1:
                    mm2_last(c)
            else:
                (mm1 if kind == 1 else mm2)(c, j)

    @pl.when(zero[2] == 1)
    def _():
        for i in range(PAD):
            a = ebuf[8 * (i % 100):8 * (i % 100) + 8, :]
            for _ in range(8):
                a = a * a + 1.0
            ebuf[8 * (i % 100):8 * (i % 100) + 8, :] = a

    for c in range(NC):
        for _, cp in out_copies(c):
            cp.wait()


@jax.jit
def pallas_sequential_preLN__ssm_conv_h3__mixer_channel_mlp__prompt_kernel(
        A_q, A_k, A_v, A_shift_k, A_ssm_k, A_ssm_D, B_x, B_w1, B_b1, B_w2, B_b2):
    qT, kT, vT = A_q[0].T, A_k[0].T, A_v[0].T
    anyspec = pl.BlockSpec(memory_space=pl.ANY)
    out = pl.pallas_call(
        _kernel,
        out_shape=jax.ShapeDtypeStruct((D, S), bf16),
        in_specs=[anyspec] * 10,
        out_specs=anyspec,
        scratch_shapes=[
            pltpu.VMEM((D, S), bf16), pltpu.VMEM((D, S), bf16), pltpu.VMEM((D, S), bf16), pltpu.VMEM((D, S), bf16),
            pltpu.VMEM((KP, F), bf16), pltpu.VMEM((F // 2, KP), u32), pltpu.VMEM((D, F), bf16),
            pltpu.VMEM((6, D, 128), f32),
            pltpu.VMEM((2 * D, 2 * B), f32),
            *[pltpu.VMEM((D, HL), f32)] * (NC - 1),
            pltpu.VMEM((D, 2 * B), f32), pltpu.VMEM((R, D + 8, 128), f32), pltpu.VMEM((D // 2, 384), u32),
            pltpu.VMEM((KP // 2 + 8, B), u32), pltpu.VMEM((KP // 2 + 8, B), u32),
            pltpu.VMEM((R, D + 8, 128), f32), pltpu.VMEM((R, D + 8, 128), f32),
            pltpu.VMEM((D, S), bf16),
            pltpu.VMEM((4, D), bf16), pltpu.VMEM((D,), bf16), pltpu.VMEM((F,), bf16), pltpu.VMEM((D,), bf16),
            pltpu.VMEM((R, 64, 256), u32), pltpu.VMEM((R, 128, 128), u32),
            pltpu.SemaphoreType.DMA((48,)), pltpu.SemaphoreType.REGULAR,
        ],
        compiler_params=pltpu.CompilerParams(vmem_limit_bytes=100 * 1024 * 1024),
    )(qT, kT, vT, A_shift_k.T, A_ssm_k, A_ssm_D, B_w1, B_b1, B_w2.T, B_b2)
    return out.T[None]
```

```python
import jax
import jax.numpy as jnp
import jax.experimental.pallas as pl
import jax.experimental.pallas.tpu as pltpu

S, D, F = 2048, 448, 1792
B = 512
R = 4
NC = S // B
KP = 512
FC = 128
NF = F // FC
RT = 16
NT = D // RT
H = RT // 2
GB = [112] * 4
G0 = [32, 48, 48, 48, 64, 64, 64, 48, 32]
ORDER0 = 'a0 a1 c0 a2 c1 a3 | c2 a4 c3 a5 c4 a6 c5 a7 c6 a8 c7 c8'
RA = 176
OG = 7
NJ0 = 7
EB0 = [0.0, 0.18, 0.5, 0.7, 0.9]
EG0 = 4
NPT = 32
GROUPS = [('par',), ('c0a',), ('c0b',), ('q0', 'w0'), ('c1', 'w1'), ('w2', 'q1'), ('c2',), ('q2', 'c3'), ('q3',)]
EPS = 1e-5
f32 = jnp.float32
bf16 = jnp.bfloat16
u32 = jnp.uint32
C1 = 0.7978845608028654
C2 = C1 * 0.044715
SK, SU = 0, 8
HL = 17 * 128
SEQ0 = ('1.0 1.1 1.2 1.3 1.4 1.5 1.6 2.0 1.7 2.1 1.8 1.9 2.2 2.3 2.4 2.5 2.6 2.7 2.8 2.9 '
        '1.10 1.11 2.10 1.12 2.11 1.13 2.12 2.13')
POS_C1 = 9
POS_AB = [12, 3, 3]
POS_D = [18, 21, 21]
POS_FD = 19
WP = [((0, 8), (0, 1)), ((8, 14), (1, 5)), ((14, 14), (5, 14))]


def _cos2048(x):
    n = x - 2048.0 * jnp.floor(x * (1.0 / 2048.0))
    u = jnp.abs(n - 1024.0) * (1.0 / 512.0) - 1.0
    u2 = u * u
    pl_ = 1.6044118478735982e-04
    for cf in (-4.681754135318688e-03, 7.969262624616703e-02, -6.459640975062462e-01, 1.5707963267948966):
        pl_ = pl_ * u2 + cf
    return pl_ * u


def _sample_index(b, p):
    r = (b - p) & 3
    return 128 * r + ((b - r) & 127)


def _bfly(e, sign):
    ar, ai = e[0][0] + e[2][0], e[0][1] + e[2][1]
    br, bi = e[0][0] - e[2][0], e[0][1] - e[2][1]
    cr, ci = e[1][0] + e[3][0], e[1][1] + e[3][1]
    dr, di = e[1][0] - e[3][0], e[1][1] - e[3][1]
    o0 = (ar + cr, ai + ci)
    o2 = (ar - cr, ai - ci)
    pm = (br - di, bi + dr)
    mm = (br + di, bi - dr)
    return [o0, pm, o2, mm] if sign > 0 else [o0, mm, o2, pm]


def _lane(shape):
    return jax.lax.broadcasted_iota(jnp.int32, shape, 1)


def _sel4(xt):
    lane4 = _lane(xt[0].shape) & 3
    odd = (lane4 & 1) == 1
    a = [[jnp.where(odd, xt[2 * r1 + 1], xt[2 * r1]) for r1 in range(2)],
         [jnp.where(odd, xt[2 * r1], xt[2 * r1 + 1]) for r1 in range(2)]]
    out = []
    for p in range(4):
        hi = ((lane4 - p) & 3) >= 2
        out.append(jnp.where(hi, a[p & 1][1], a[p & 1][0]))
    return out


def _cmul(k, u):
    return k[0] * u[0] - k[1] * u[1], k[0] * u[1] + k[1] * u[0]


def _pack(x):
    return pltpu.bitcast(x.astype(bf16), u32)


def _unpk(w):
    return pltpu.bitcast(w, bf16).astype(f32)


class _Stats:
    def __init__(self, nacc=1):
        self.piv = None
        self.a1 = [None] * nacc
        self.a2 = [None] * nacc
        self.k = 0

    def add(self, x, use_pivot=True):
        if use_pivot:
            if self.piv is None:
                self.piv = jnp.broadcast_to(x[0:1, :], (8, x.shape[1]))
        for i in range(x.shape[0] // 8):
            d = x[8 * i:8 * (i + 1), :]
            if use_pivot:
                d = d - self.piv
            k = self.k % len(self.a1)
            self.k += 1
            self.a1[k] = d if self.a1[k] is None else self.a1[k] + d
            self.a2[k] = d * d if self.a2[k] is None else self.a2[k] + d * d
        self.s1, self.s2 = self.a1[0], self.a2[0]

    def finish(self):
        s1, s2 = sum(self.a1[1:], self.a1[0]), sum(self.a2[1:], self.a2[0])
        n = s1.shape[1]
        e1 = jnp.sum(s1, axis=0, keepdims=True) * (1.0 / D)
        e2 = jnp.sum(s2, axis=0, keepdims=True) * (1.0 / D)
        var = jnp.maximum(e2 - e1 * e1, 0.0)
        mean = e1 if self.piv is None else e1 + self.piv[0:1, :]
        rstd = jax.lax.rsqrt(var + EPS)
        return jnp.broadcast_to(mean, (8, n)), jnp.broadcast_to(rstd, (8, n))


def _rep(a, n):
    return jnp.concatenate([a] * n, axis=0)


def _kernel(q_hbm, k_hbm, v_hbm, sh_hbm, sk_hbm, sd_hbm, w1_hbm, b1_hbm, w2_hbm, b2_hbm,
            out_hbm,
            qb, kb, vb, skb, w1b, w1t, w2b, par, ebuf, hc0, hc1, hc2, vbuf, ybuf, halo,
            xn0, xn1, hres0, hres1, ob, sh_ref, sd_ref, b1_ref, b2_ref, fm_ref, gm_ref,
            sems, fsem):
    xn = [xn0, xn1]
    hres = [hres0, hres1]
    hc = [hc0, hc1, hc2]

    copies = {}

    def add(name, src, dst):
        si = [i for i, grp in enumerate(GROUPS) if name in grp][0]
        copies.setdefault(name, []).append(pltpu.make_async_copy(src, dst, sems.at[si]))

    def cols(ref, lo, n, rows=None):
        return ref.at[:, pl.ds(lo, n)] if rows is None else ref.at[pl.ds(rows[0], rows[1]), pl.ds(lo, n)]

    def add_conv(name, c, rows=None):
        for src, dst in ((k_hbm, kb), (v_hbm, vb), (sk_hbm, skb)):
            add(name, cols(src, c * B, B, rows), cols(dst, c * B, B, rows))

    def add_w(i):
        (a0, a1), (b0, b1) = WP[i]
        if a1 > a0:
            add('w%d' % i, cols(w1_hbm, a0 * FC, (a1 - a0) * FC), cols(w1b, a0 * FC, (a1 - a0) * FC, (0, D)))
        if b1 > b0:
            add('w%d' % i, cols(w2_hbm, b0 * FC, (b1 - b0) * FC), cols(w2b, b0 * FC, (b1 - b0) * FC))

    for src, dst in ((sh_hbm, sh_ref), (sd_hbm, sd_ref), (b2_hbm, b2_ref), (b1_hbm, b1_ref)):
        add('par', src, dst)
    add_conv('c0a', 0, (0, RA))
    add_conv('c0b', 0, (RA, D - RA))
    add('q0', cols(q_hbm, 0, B), cols(qb, 0, B))
    add_w(0)
    add_conv('c1', 1)
    add_w(1)
    add_w(2)
    for c in range(1, NC):
        add('q%d' % c, cols(q_hbm, c * B, B), cols(qb, c * B, B))
        if c + 1 < NC:
            add_conv('c%d' % (c + 1), c + 1)
    for lst in copies.values():
        for cp in lst:
            cp.start()

    def wait(*names):
        assert not names or names in GROUPS
        if not names:
            pl.semaphore_signal(fsem, 1)
            pl.semaphore_wait(fsem, 1)
        for nm in names:
            for cp in copies.pop(nm):
                cp.wait()

    def out_copy(c):
        return pltpu.make_async_copy(cols(ob, c * B, B), cols(out_hbm, c * B, B), sems.at[0])

    def out_copy_last(hf, g):
        gr = D // OG
        c0 = pl.multiple_of((NC - 1) * B + hf * (B // 2), B // 2)
        return pltpu.make_async_copy(cols(ob, c0, B // 2, (g * gr, gr)), cols(out_hbm, c0, B // 2, (g * gr, gr)),
                                     sems.at[0])

    def make_fm(p):
        t = _sample_index(jax.lax.broadcasted_iota(jnp.int32, (128, 128), 0), p).astype(f32)
        x = t * (4 * jax.lax.broadcasted_iota(jnp.int32, (128, 128), 1) + 1).astype(f32)
        toks = []
        for z in range(2):
            w = _pack(_cos2048(x + 512.0 * z))
            fm_ref[p, :, 128 * z:128 * (z + 1)] = w
            toks += [w[8 * i:8 * (i + 1), :] for i in range(8)]
        return toks

    def make_gm(p):
        gm_ref[p] = pltpu.bitcast(pltpu.bitcast(fm_ref[p], bf16).T, u32)

    wait()
    for p in (0, 2):
        make_fm(p)
    wait('par')
    i0 = jax.lax.broadcasted_iota(jnp.int32, (8, 128), 0)
    i1 = jax.lax.broadcasted_iota(jnp.int32, (8, 128), 1)
    zero = [jnp.min(a.astype(f32)).astype(jnp.int32) for a in (i0 + i1, i1, 2 * i1 + i0)]
    z8 = pl.multiple_of(jnp.clip(8 * zero[0], 0, 8), 8)
    never = [i1 < zero[1 + i] for i in range(2)]

    def dview(ref):
        n = ref.shape[-2] - 8
        return ref.at[pl.ds(z8, n), :] if len(ref.shape) == 2 else ref.at[:, pl.ds(z8, n), :]

    ybuf_w = dview(ybuf)
    xn_w = [dview(a) for a in xn]
    hres_w = [dview(a) for a in hres]

    P = jnp.concatenate([sh_ref[...].astype(f32), sd_ref[...].astype(f32).reshape(1, D),
                         b2_ref[...].astype(f32).reshape(1, D), jnp.zeros((2, D), f32)], axis=0)
    Pp = jnp.concatenate([P, jnp.zeros((8, 64), f32)], axis=1)
    PT = jnp.concatenate([Pp] * 16, axis=0).T

    gtok = make_fm(1) + make_fm(3)
    ptile = []
    for i in range(D // 8):
        w = PT[8 * i:8 * (i + 1), :]
        for q, t in enumerate(gtok[i * len(gtok) // NPT:(i + 1) * len(gtok) // NPT]):
            w = jnp.where(never[q % 2], pltpu.bitcast(t, f32), w)
        ptile.append(w)
    plhs = jnp.concatenate(ptile, axis=0).astype(bf16)
    for p in (0, 2, 1, 3):
        make_gm(p)

    def set_par(j0, j1):
        n = 128 * (j1 - j0)
        onehot = (jax.lax.broadcasted_iota(jnp.int32, (128, n), 0)
                  == j0 + jax.lax.broadcasted_iota(jnp.int32, (128, n), 1) // 128)
        pb = jnp.dot(plhs, jnp.where(onehot, 1.0, 0.0).astype(bf16), preferred_element_type=f32)
        for j in range(j0, j1):
            par[j] = pb[:, 128 * (j - j0):128 * (j - j0 + 1)]

    set_par(0, 4)
    rowx = jax.lax.broadcasted_iota(jnp.int32, ((KP - D) // 2, B), 0)
    ones_rows = jnp.where(rowx == 0, jnp.uint32(0x3F80), jnp.uint32(0))
    for i in range(2):
        xn[i][D // 2:KP // 2, :] = ones_rows
    b1row = b1_ref[...].astype(f32).reshape(1, F)

    row = jax.lax.broadcasted_iota(jnp.int32, (KP - D, F), 0)
    w1b[D:KP, :] = jnp.where(row == 0, jnp.broadcast_to(b1row, (KP - D, F)), 0.0).astype(bf16)

    def prep_w(a0, a1):
        for j in range(a0, a1):
            w1t[j * FC // 2:(j + 1) * FC // 2, :] = pltpu.bitcast(w1b[0:KP, j * FC:(j + 1) * FC].T, u32)

    st = {}

    def slot(s):
        return slice(128 * s, 128 * (s + 1))

    def shuffle(blocks):
        return _sel4([blocks[0]] + [pltpu.roll(blocks[r], r, 1) for r in range(1, R)])

    def fwd(c, t0, nt):
        rows = slice(RT * t0, RT * (t0 + nt))
        wrows = slice(H * t0, H * (t0 + nt))
        lane = _lane((H * nt, 128))
        taps = [par[s, rows, :] for s in range(4)]
        if c == 0:
            prev = [jnp.zeros((H * nt, 128), u32)] * 3
        else:
            prev = [halo[wrows, slot(s)] for s in range(3)]
        pk = shuffle([pltpu.bitcast(skb[rows, c * B + 128 * r:c * B + 128 * (r + 1)], u32) for r in range(R)])
        ub = []
        for r in range(R):
            ls = slice(c * B + 128 * r, c * B + 128 * (r + 1))
            kw = pltpu.bitcast(kb[rows, ls], u32)
            cur = [pltpu.roll(kw, s, 1) for s in range(1, 4)]
            ks = [kw] + [jnp.where(lane >= s, cur[s - 1], prev[s - 1]) for s in range(1, 4)]
            prev = cur
            acc = (_unpk(ks[0]) * taps[0] + _unpk(ks[1]) * taps[1]) + (
                _unpk(ks[2]) * taps[2] + _unpk(ks[3]) * taps[3])
            ub.append(_pack(acc * vb[rows, ls].astype(f32)))
        if c < NC - 1:
            for s in range(3):
                halo[wrows, slot(s)] = prev[s]
        pu = shuffle(ub)
        e = [None] * R
        for p in (0, 2, 1, 3):
            w = jnp.concatenate([pk[p].reshape(nt, H, 128), pu[p].reshape(nt, H, 128)], axis=1)
            lhs = pltpu.bitcast(w.reshape(RT * nt, 128), bf16)
            e[p] = jnp.dot(lhs, pltpu.bitcast(fm_ref[p], bf16), preferred_element_type=f32).reshape(nt, 2 * RT, 256)
        return e

    def stage_ab(c):
        t0 = 0
        for gr in GB:
            e = fwd(c, t0, gr // RT)
            for p in range(R):
                ebuf[t0:t0 + gr // RT, :, 256 * p:256 * (p + 1)] = e[p]
            t0 += gr // RT

    def ld(ar, rows, s0):
        return [(ar[rows, slot(s0 + 2 * m)], ar[rows, slot(s0 + 2 * m + 1)]) for m in range(R)]

    def sto(ar, rows, s0, vals):
        for m in range(R):
            ar[rows, slot(s0 + 2 * m)] = vals[m][0]
            ar[rows, slot(s0 + 2 * m + 1)] = vals[m][1]

    def stage_c(c, t0, nt, e):
        rows = slice(RT * t0, RT * (t0 + nt))
        ek, eu = [[tuple(e[p][:, o:o + RT, slot(z)].reshape(RT * nt, 128) for z in range(2)) for p in range(R)]
                  for o in (0, RT)]
        km = _bfly(ek, -1)
        dd = par[4, rows, :]
        kold = [ld(hc[cc], rows, SK) for cc in range(c)]
        uold = [ld(hc[cc], rows, SU) for cc in range(c)]
        if c == 0:
            kc = [(km[m][0] + dd, km[m][1]) for m in range(R)]
        else:
            kprev = [(a - dd, b) for a, b in kold[0]]
            for cc in range(1, c):
                kprev = [(kold[cc][m][0] + kprev[m][1], kold[cc][m][1] - kprev[m][0]) for m in range(R)]
            kc = [(km[m][0] - kprev[m][1], km[m][1] + kprev[m][0]) for m in range(R)]
        um = _bfly(eu, -1)
        if c < NC - 1:
            sto(hc[c], rows, SK, kc)
            sto(hc[c], rows, SU, um)
        ks, us = kold + [kc], uold + [um]
        ym = []
        for m in range(R):
            y = None
            for dl in range(c + 1):
                tt = _cmul(ks[dl][m], us[c - dl][m])
                y = tt if y is None else (y[0] + tt[0], y[1] + tt[1])
            ym.append(y)
        return ym, _bfly(ym, +1)

    def stage_c_all(c):
        ym, vp = stage_c(c, 0, NT, [ebuf[:, :, 256 * p:256 * (p + 1)] for p in range(R)])
        sto(vbuf, slice(0, D), 0, vp)
        ym, vp = [[[pltpu.bitcast(a, u32) for a in x] for x in arr] for arr in (ym, vp)]
        toks = []
        for i in range(D // 8):
            rows = slice(8 * i, 8 * (i + 1))
            for m in (0, 2, 1, 3):
                toks += [(ym[m][0][rows, :], 6 * c + 3 + (14 if m < 2 else 6)), (ym[m][1][rows, :], 4 * (c + 1))]
            toks += [(vp[p][z][rows, :], 3) for p in (0, 2, 1, 3) for z in range(2)]
        return toks

    def inv(v, t0, nt, dst):
        xt = _sel4([jnp.dot(v[p].astype(bf16), pltpu.bitcast(gm_ref[p], bf16), preferred_element_type=f32)
                    for p in range(R)])
        for r in range(R):
            dst[r, RT * t0:RT * (t0 + nt), :] = xt[r] if r == 0 else pltpu.roll(xt[r], 128 - r, 1)

    def stage_d(c):
        inv([vbuf[:, 256 * p:256 * (p + 1)] for p in range(R)], 0, NT, ybuf_w if c > 1 else ybuf)

    def gate(a, i, on):
        return jax.lax.select(never[0], par[i // 56, 8 * (i % 56):8 * (i % 56) + 8, :], a) if on else a

    def stage_x(c, r):
        toks = []
        s = _Stats(4 if c == 0 and r == 0 else 1)
        for t in range(D // 32):
            s.add(qb[t * 32:(t + 1) * 32, c * B + 128 * r:c * B + 128 * (r + 1)].astype(f32))
            toks += [(s.s1, 13), (s.s2, 9)]
        st['xs', c, r] = s.finish()
        return toks

    def stage_e1(c, r):
        hr = hres[c % 2]
        toks = []
        mx, rx = st.pop(('xs', c, r))
        mx, rx = _rep(mx, 2), _rep(rx * (1.0 / B), 2)
        s = _Stats(4 if c == 0 and r == 0 else 1)
        for t in range(NT):
            rows = slice(t * RT, (t + 1) * RT)
            x = qb[rows, c * B + 128 * r:c * B + 128 * (r + 1)].astype(f32)
            y = ybuf[r, rows, :]
            h = x + (x - mx) * rx * y
            (hres_w[c % 2] if c > 1 else hr)[r, rows, :] = h
            s.add(h)
            toks += [(s.s1, 15), (s.s2, 5)]
        st['hs', r] = s.finish()
        return toks

    def stage_e2(c, r, gt):
        hr = hres[c % 2]
        toks = []
        m1, r1 = st['hs', r]
        r1 = _rep(r1, 4)
        s = _Stats(4 if c == 0 and r == 0 else 1)
        for t in range(D // 32):
            m1g = _rep(gate(m1, 14 * r + t, gt), 4)
            s.add((hr[r, t * 32:(t + 1) * 32, :] - m1g) * r1, use_pivot=False)
            toks += [(s.s1, 14), (s.s2, 9)]
        st['ns', r] = s.finish()
        return toks

    def stage_e3(c, r, gt):
        hr = hres[c % 2]
        toks = []
        (m1, r1), (m2, r2) = st.pop(('hs', r)), st.pop(('ns', r))
        r1, m2, r2 = _rep(r1, 2), _rep(m2, 2), _rep(r2, 2)
        for t in range(NT):
            if t % 2 == 0:
                m1g = _rep(gate(m1, 56 + 14 * r + t // 2, gt), 2)
            w = _pack(((hr[r, t * RT:(t + 1) * RT, :] - m1g) * r1 - m2) * r2)
            (xn_w if c > 1 else xn)[c % 2][t * H:(t + 1) * H, slot(r)] = w
            toks.append((w, 14))
        return toks

    def hld(hr):
        return jnp.concatenate([hr[r, 0:D, :] for r in range(R)], axis=1)

    pts = {}

    def attach(col, keys):
        if not any(k in pts for k in keys):
            return col
        tiles = []
        for i, key in enumerate(keys):
            w = col[H * i:H * (i + 1), :]
            for q, t in enumerate(pts.pop(key, ())):
                w = jax.lax.select(never[q % 2], t if t.dtype == u32 else pltpu.bitcast(t, u32), w)
            tiles.append(w)
        return jnp.concatenate(tiles, axis=0)

    def up_proj(c, r0, nr, keys):
        zs = []
        for n in range(R):
            w = jnp.concatenate([attach(w1t[r0:r0 + nr, 0:128], keys(n)), w1t[r0:r0 + nr, 128:]], axis=1)
            zs.append(jnp.dot(pltpu.bitcast(w, bf16), pltpu.bitcast(xn[c % 2][0:KP // 2, slot(n)], bf16),
                              preferred_element_type=f32))
        return jnp.concatenate(zs, axis=1)

    def mm1(c, j):
        if any(k[:3] == (c, 1, j) for k in pts):
            z = up_proj(c, j * FC // 2, FC // 2, lambda n: [(c, 1, j, n, i) for i in range(FC // RT)])
        else:
            lhs = pltpu.bitcast(w1t[j * FC // 2:(j + 1) * FC // 2, :], bf16)
            z = jnp.dot(lhs, pltpu.bitcast(xn[c % 2][0:KP // 2, :], bf16), preferred_element_type=f32)
        gelu(z, j)

    def gelu(z, j):
        t = jnp.tanh(z * (C1 + C2 * (z * z)))
        hz = 0.5 * z
        st['ht', j] = (hz + hz * t).astype(bf16)

    def mm1_first(c, nj):
        z = up_proj(c, 0, nj * FC // 2, lambda n: [(c, 3, n, i) for i in range(nj * FC // RT)])
        for j in range(nj):
            gelu(z[j * FC:(j + 1) * FC, :], j)

    def mm2(c, j):
        lhs = w2b[:, j * FC:(j + 1) * FC]
        if any((c, 2, j, i) in pts for i in range(NT)):
            lhs = pltpu.bitcast(attach(pltpu.bitcast(lhs, u32), [(c, 2, j, i) for i in range(NT)]), bf16)
        acc = hld(hres[c % 2]) + jnp.dot(lhs, st.pop(('ht', j)), preferred_element_type=f32)
        if j < NF - 1:
            for r in range(R):
                hres[c % 2][r, 0:D, :] = acc[:, slot(r)]
        else:
            acc = acc + jnp.concatenate([par[5]] * R, axis=1)
            ob[:, pl.ds(c * B, B)] = acc.astype(bf16)
            out_copy(c).start()

    def mlp_last(hf, carry):
        c = NC - 1
        f2 = 2 * FC
        xh = pltpu.bitcast(xn[c % 2][0:KP // 2, pl.ds(pl.multiple_of(hf * (B // 2), B // 2), B // 2)], bf16)

        def up(j):
            gelu(jnp.dot(pltpu.bitcast(w1t[j * FC:(j + 1) * FC, :], bf16), xh, preferred_element_type=f32), j)

        acc = jnp.concatenate([hres[c % 2][2 * hf + r, 0:D, :] + par[5] for r in range(2)], axis=1)
        up(1)
        for j in range(1, F // f2):
            if j + 1 < F // f2:
                up(j + 1)
            acc = acc + jnp.dot(w2b[:, j * f2:(j + 1) * f2], st.pop(('ht', j)), preferred_element_type=f32)
        gr = D // OG
        for g in range(OG):
            ob[g * gr:(g + 1) * gr, pl.ds(pl.multiple_of(c * B + hf * (B // 2), B // 2), B // 2)] = (
                acc[g * gr:(g + 1) * gr, :].astype(bf16))
            out_copy_last(hf, g).start()
        return carry

    seq = [(1, 0)] + [x for j in range(NF) for x in ([(1, j + 1)] if j + 1 < NF else []) + [(2, j)]]

    seq0 = [(int(x.split('.')[0]), int(x.split('.')[1])) for x in SEQ0.split()]
    seqs = [seq0, seq, seq]

    def points(c, i0, i1):
        out = []
        for kind, j in seqs[c][i0:i1]:
            if kind == 1:
                out += [(c, 1, j, n, i) for n in range(R) for i in range(FC // RT)]
            else:
                out += [(c, 2, j, i) for i in range(NT)]
        return out

    def place(toks, keys):
        total = sum(w for _, w in toks)
        acc = 0
        for t, w in toks:
            acc += w
            k = min(len(keys) - 1, (acc * len(keys) - 1) // total)
            pts.setdefault(keys[k], []).append(t)

    go = [sum(G0[:g]) // RT for g in range(len(G0))]

    def c0_ab(g):
        st['e', g] = fwd(0, go[g], G0[g] // RT)

    def c0_cd(g):
        _, vp = stage_c(0, go[g], G0[g] // RT, st.pop(('e', g)))
        inv([jnp.concatenate(vp[p], axis=1) for p in range(R)], go[g], G0[g] // RT, ybuf)

    wait('c0a')
    set_par(4, 6)
    for ev in ORDER0.split():
        if ev == '|':
            wait('c0b')
        else:
            (c0_ab if ev[0] == 'a' else c0_cd)(int(ev[1]))
    wait('q0', 'w0')
    prep_w(0, NJ0)
    for r in range(R):
        tk = [stage_x(0, r), stage_e1(0, r), stage_e2(0, r, r > 0), stage_e3(0, r, r > 0)]
        if r > 0:
            keys = [(0, 3, r - 1, i) for i in range(NJ0 * FC // RT)]
            b = [int(len(keys) * x) for x in EB0]
            for q in range(4):
                place(tk[q], keys[b[q] + (EG0 if q else 2):b[q + 1]])
    fence_ab = [None, ('w2', 'q1'), ('q2', 'c3'), ('q3',)]
    for c in range(NC - 1):
        n = c + 1
        for i, (kind, j) in enumerate(seqs[c]):
            if c == 0 and i == POS_C1:
                wait('c1', 'w1')
            if n < NC and i == POS_AB[c]:
                stage_ab(n)
                wait(*fence_ab[n])
                keys = points(c, i, POS_D[c])[6:-4]
                place(stage_c_all(n), keys)
                if n > 1:
                    place([x for r in range(R) for x in stage_x(n, r)], keys)
            if n < NC and i == POS_D[c]:
                stage_d(n)
                if n >= 2:
                    for r in range(R):
                        stage_e1(n, r)
                    for r in range(R):
                        stage_e2(n, r, False)
                    for r in range(R):
                        stage_e3(n, r, False)
            if c == 0 and i == POS_FD:
                wait('c2')
                keys = points(c, i, len(seq) - 1)
                b = [int(len(keys) * x) for x in [0.0, 0.2, 0.56, 0.78, 1.0]]
                place([x for r in range(R) for x in stage_x(n, r)], keys[6:b[1]])
                place([x for r in range(R) for x in stage_e1(n, r)], keys[b[1] + 6:b[2]])
                place([x for r in range(R) for x in stage_e2(n, r, True)], keys[b[2] + 8:b[3]])
                place([x for r in range(R) for x in stage_e3(n, r, True)], keys[b[3] + 8:b[4]])
            if c == 0 and kind == 1 and j < NJ0:
                if j == 0:
                    mm1_first(0, NJ0)
            else:
                if c == 0 and kind == 1:
                    prep_w(j, j + 1)
                (mm1 if kind == 1 else mm2)(c, j)
    mm1(NC - 1, 0)
    mm1(NC - 1, 1)
    mm2(NC - 1, 0)
    mm2(NC - 1, 1)
    jax.lax.fori_loop(0, 2, mlp_last, 0)
    for c in range(NC - 1):
        out_copy(c).wait()
    for hf in range(2):
        for g in range(OG):
            out_copy_last(hf, g).wait()


@jax.jit
def pallas_sequential_preLN__ssm_conv_h3__mixer_channel_mlp__prompt_kernel(
        A_q, A_k, A_v, A_shift_k, A_ssm_k, A_ssm_D, B_x, B_w1, B_b1, B_w2, B_b2):
    qT, kT, vT = A_q[0].T, A_k[0].T, A_v[0].T
    anyspec = pl.BlockSpec(memory_space=pl.ANY)
    out = pl.pallas_call(
        _kernel,
        out_shape=jax.ShapeDtypeStruct((D, S), bf16),
        in_specs=[anyspec] * 10,
        out_specs=anyspec,
        scratch_shapes=[
            pltpu.VMEM((D, S), bf16), pltpu.VMEM((D, S), bf16), pltpu.VMEM((D, S), bf16), pltpu.VMEM((D, S), bf16),
            pltpu.VMEM((KP, F), bf16), pltpu.VMEM((F // 2, KP), u32), pltpu.VMEM((D, F), bf16),
            pltpu.VMEM((6, D, 128), f32),
            pltpu.VMEM((NT, 2 * RT, 2 * B), f32),
            *[pltpu.VMEM((D, HL), f32)] * (NC - 1),
            pltpu.VMEM((D, 2 * B), f32), pltpu.VMEM((R, D + 8, 128), f32), pltpu.VMEM((D // 2, 384), u32),
            pltpu.VMEM((KP // 2 + 8, B), u32), pltpu.VMEM((KP // 2 + 8, B), u32),
            pltpu.VMEM((R, D + 8, 128), f32), pltpu.VMEM((R, D + 8, 128), f32),
            pltpu.VMEM((D, S), bf16),
            pltpu.VMEM((4, D), bf16), pltpu.VMEM((D,), bf16), pltpu.VMEM((F,), bf16), pltpu.VMEM((D,), bf16),
            pltpu.VMEM((R, 64, 256), u32), pltpu.VMEM((R, 128, 128), u32),
            pltpu.SemaphoreType.DMA((len(GROUPS),)), pltpu.SemaphoreType.REGULAR,
        ],
        compiler_params=pltpu.CompilerParams(vmem_limit_bytes=100 * 1024 * 1024, disable_bounds_checks=True,
                                             disable_semaphore_checks=True),
    )(qT, kT, vT, A_shift_k.T, A_ssm_k, A_ssm_D, B_w1, B_b1, B_w2.T, B_b2)
    return out.T[None]
```
